```python
import os as _os
_os.environ.setdefault("JAX_PLATFORMS", "cpu")
import jax
import jax.numpy as jnp

def _softmax(x, axis=-1):
    return jax.nn.softmax(x, axis=axis)
def _gelu(x):
    return jax.nn.gelu(x, approximate=True)
def _silu(x):
    return jax.nn.silu(x)
def _sigmoid(x):
    return jax.nn.sigmoid(x)
def _layernorm(x, axis=-1, eps=1e-5):
    m = jnp.mean(x, axis=axis, keepdims=True)
    v = jnp.var(x, axis=axis, keepdims=True)
    return (x - m) / jnp.sqrt(v + eps)
def _scatter_add(tgt, idx, src, axis=0):
    return tgt.at[idx].add(src)
def _segment_sum(src, seg, n):
    return jax.ops.segment_sum(src, seg, n)
class _Rng:
    def __init__(self, key):
        self._k = key
    def _next(self):
        self._k, sub = jax.random.split(self._k)
        return sub
    def normal(self, shape):
        return jax.random.normal(self._next(), shape, dtype=jnp.bfloat16)
    def randint(self, lo, hi, shape):
        return jax.random.randint(self._next(), shape, lo, hi, dtype=jnp.int32)
    def uniform(self, shape, lo=0.0, hi=1.0):
        return jax.random.uniform(self._next(), shape, jnp.bfloat16, lo, hi)
    def permutation(self, n):
        return jax.random.permutation(self._next(), n)


kernel_name = 'sequential_preLN__sliding_block__dense_activation_relu__prompt'

def setup_inputs():
    _rng = _Rng(jax.random.key(int.from_bytes(__import__("os").urandom(4), "little")))
    _w = (lambda a: (lambda t: t.astype(jnp.bfloat16) if jnp.issubdtype(t.dtype, jnp.floating) else t)(jnp.asarray(a)))
    def _A_setup():
        B, S, D = 1, 2048, 640
        return {
            "x": _w((lambda *s: _rng.normal(s) * 0.05)(B, S, D)),
            "wqkv": _w((lambda *s: _rng.normal(s) * 0.05)(D, 3 * D)),
            "wo": _w((lambda *s: _rng.normal(s) * 0.05)(D, D)),
        }
    _A_in = _A_setup()

    def _B_setup():
        B, S, D, Dff = 1, 2048, 640, 1536
        return {
            "x": _w((lambda *s: _rng.normal(s) * 0.05)(B, S, D)),
            "w1": _w((lambda *s: _rng.normal(s) * 0.05)(D, Dff)),
            "w2": _w((lambda *s: _rng.normal(s) * 0.05)(Dff, D)),
        }
    _B_in = _B_setup()

    return {
        "A_x": _A_in["x"],
        "A_wqkv": _A_in["wqkv"],
        "A_wo": _A_in["wo"],
        "B_x": _B_in["x"],
        "B_w1": _B_in["w1"],
        "B_w2": _B_in["w2"],
    }

def reference(A_x, A_wqkv, A_wo, B_x, B_w1, B_w2):
    def _A_ref(x, wqkv, wo):
        B, S, D = x.shape
        H = 32; Dh = D // H; W = 256
        qkv = (lambda x, *d: x.transpose(*d))((x @ wqkv).reshape(B, S, 3, H, Dh), 2, 0, 3, 1, 4)
        q, k, v = qkv[0], qkv[1], qkv[2]
        scores = jnp.einsum("bhqd,bhkd->bhqk", q, k) * (Dh ** -0.5)
        idx = jnp.arange(S)
        mask = (idx[:, None] - idx[None, :] >= 0) & (idx[:, None] - idx[None, :] < W)
        scores = jnp.where(mask[None, None], scores, -1e9)
        p = _softmax(scores, axis=-1)
        o = jnp.einsum("bhqk,bhkd->bhqd", p, v)
        return (lambda x, *d: x.transpose(*d))(o, 0, 2, 1, 3).reshape(B, S, D) @ wo

    def _B_ref(x, w1, w2):
        h = jnp.einsum("bsd,df->bsf", x, w1)
        zero = jnp.zeros_like(h)
        h = jnp.maximum(h, zero)
        return jnp.einsum("bsf,fd->bsd", h, w2)

    x = A_x
    h = x + _A_ref(_layernorm(x, axis=-1), A_wqkv, A_wo)
    h2 = h + _B_ref(_layernorm(h, axis=-1), B_w1, B_w2)
    return h2
```

```python
import functools
import os as _os
import math

import jax
import jax.numpy as jnp
from jax import lax
import jax.experimental.pallas as pl
import jax.experimental.pallas.tpu as pltpu

H = 32
W = 256
QT = 128
L = 128
EPS = 1e-5
NEG = -3.0e38
T = 256
G = 4
NG = H // G
VR = 24
QB = 32
FR = 128
F1 = 4
LAG = int(_os.environ.get('LAG', 3))
LAG0 = int(_os.environ.get('LAG0', 3))
NB = max(LAG, LAG0) + 1
FENCE = int(_os.environ.get('FENCE', 1))
LNF = int(_os.environ.get('LNF', 0))
FT = int(_os.environ.get('FT', 3))
FPOS = [int(c) for c in _os.environ.get('FPOS', '0,2,5,8,11,13,14,15').split(',')]
EARLY = int(_os.environ.get('EARLY', 1))
LT1 = int(_os.environ.get('LT1', 4))
LT2 = int(_os.environ.get('LT2', 2))

_NT = (((1,), (1,)), ((), ()))


def _layernorm_f32(x):
    m = jnp.mean(x, axis=-1, keepdims=True)
    xc = x - m
    v = jnp.mean(xc * xc, axis=-1, keepdims=True)
    return xc * lax.rsqrt(v + EPS)


def _b16(x):
    return pltpu.bitcast(x, jnp.bfloat16)


def _pack16(a):
    r, c = a.shape
    a3 = a.reshape(r // 16, 16, c)
    lo = a3[:, 0:8, :].reshape(r // 2, c)
    hi = a3[:, 8:16, :].reshape(r // 2, c)
    return pltpu.pack_elementwise([lo, hi], packed_dtype=jnp.bfloat16).astype(jnp.uint32)


def _kernel(x_hbm, wqkv_hbm, wo_hbm, w1_hbm, w2_hbm, o_hbm,
            x_scr, o_scr, wqkv_ref, wo_ref, w1_ref, w2_ref, k_scr, vt_scr, ot_scr, on_scr,
            xn_scr, xnp_scr, q_scr, hres_scr, hn_scr, a_scr, sems, xsems, osems, *sp_scrs,
            D, Dh, Dff, n):
    step = pl.program_id(0)
    nq = T // QT
    npad = W // QT
    f32, bf16 = jnp.float32, jnp.bfloat16
    qscale = (Dh ** -0.5) * math.log2(math.e)
    hq = QB // 2
    nc = W // QB
    nd = D // L
    nu = nq * NG
    P = functools.partial
    s_scrs, p_scrs = sp_scrs[:NB * G], sp_scrs[NB * G:]
    zw = step // n
    zr = step // (n + 1)
    (x_scr, o_scr, wqkv_ref, wo_ref, w1_ref, w2_ref, on_scr, xn_scr, hn_scr, a_scr) = [
        r.bitcast(bf16) for r in
        (x_scr, o_scr, wqkv_ref, wo_ref, w1_ref, w2_ref, on_scr, xn_scr, hn_scr, a_scr)]

    def xrows(i):
        return pl.ds(pl.multiple_of(i * T, T), T)

    def xcopy(i):
        return pltpu.make_async_copy(x_hbm.at[0, xrows(i)], x_scr.at[xrows(i)], xsems.at[i])

    def ocopy(i):
        rows = pl.ds(pl.multiple_of(i * FR, FR), FR)
        return pltpu.make_async_copy(o_scr.at[rows], o_hbm.at[0, rows], osems.at[i])

    qkv = lambda c0, c1: (wqkv_hbm, wqkv_ref, c0 * L, c1 * L)
    wlist = [qkv(5, 9), qkv(9, 10), qkv(0, 3), qkv(3, 5), qkv(10, 12), qkv(12, 15),
             (wo_hbm, wo_ref, 0, D), (w1_hbm, w1_ref, 0, Dff), (w2_hbm, w2_ref, 0, D)]

    def wcopy(i):
        src, dst, lo, hi = wlist[i]
        return pltpu.make_async_copy(src.at[:, lo:hi], dst.at[:, lo:hi], sems.at[i])

    def windows(tile):
        half = pl.multiple_of(tile * (T // 2), T // 2)
        k_win = k_scr.at[pl.ds(half, (W + 2 * T) // 2)]
        q_win = q_scr.at[pl.ds(half, T)]
        vt_win = vt_scr.at[pl.ds(tile * nq, npad + 2 * nq)]
        xnp_win = xnp_scr.at[pl.ds(half, T)]
        return k_win.bitcast(bf16), q_win, q_win.bitcast(bf16), vt_win, xnp_win

    def body(first, last):
        lag = LAG0 if first else LAG
        row8 = lax.broadcasted_iota(jnp.int32, (8, QT), 0)
        kk = lax.broadcasted_iota(jnp.int32, (QB, QT), 0)
        qq = lax.broadcasted_iota(jnp.int32, (QB, QT), 1) % QB
        tri = kk > qq
        tri_a = ((_pack16(jnp.where(tri, -1.0, 0.0)) >> 15) & jnp.uint32(0x00010001)
                 ) * jnp.uint32(0xFFFF)
        tri_c = ~tri_a
        lane = lax.broadcasted_iota(jnp.int32, (hq, QT), 1)
        bit0 = (lane & QB) != 0
        bit1 = (lane & (2 * QB)) != 0
        win = windows(step)

        def ln1(w, po, ref):
            xn32 = _layernorm_f32(ref[...].astype(f32))
            xn_scr[...] = xn32.astype(bf16)
            w[4][po // 2:(po + T) // 2, :] = _pack16(xn32)

        blocks = {}
        fence = {}

        def proj_qk(w, po, r0, r1, c0, c1):
            k_win, _, q16_win = w[:3]
            a = jnp.dot(xn_scr[r0:r1, :], wqkv_ref[:, c0 * L:c1 * L],
                        preferred_element_type=f32)
            for c in range(c0, c1):
                blk = a[:, (c - c0) * L:(c - c0 + 1) * L]
                blocks[r0, c] = blk * qscale if c < nd else blk
            for j in range(2 * NG):
                f0 = (j % NG) * G * Dh
                g, l0 = f0 // L + (j // NG) * nd, f0 % L
                wrap = l0 + G * Dh > L
                if not c0 <= g + wrap < c1:
                    continue
                blk = blocks[r0, g]
                if wrap:
                    ln = lax.broadcasted_iota(jnp.int32, blk.shape, 1)
                    blk = jnp.where(ln >= l0, blk, blocks[r0, g + 1])
                js = slice((j % NG) * L, (j % NG + 1) * L)
                if j < NG:
                    q16_win[po + r0:po + r1, js] = blk.astype(bf16)
                else:
                    k_win[W + po + r0:W + po + r1, js] = blk.astype(bf16)

        def proj_v(w, po, r0, r1, c0, c1):
            vt_win = w[3]
            v = jnp.dot(_b16(w[4][(po + r0) // 2:(po + r1) // 2, :]),
                        wqkv_ref[:, 2 * D + c0 * L:2 * D + c1 * L],
                        preferred_element_type=f32)
            for t in range(r0 // QT, r1 // QT):
                vt = v[t * QT - r0:(t + 1) * QT - r0, :].T
                kt = npad + po // QT + t
                for r in range((c1 - c0) * L // 8):
                    f0 = c0 * L + r * 8
                    blk = vt[r * 8:(r + 1) * 8]
                    hd = f0 // Dh
                    if (f0 + 7) // Dh == hd:
                        d0 = hd * VR + (f0 - hd * Dh + 4) // 8 * 8
                        vt_win[kt, d0:d0 + 8, :] = blk
                    else:
                        vt_win[kt, hd * VR + 16:hd * VR + 24, :] = jnp.where(
                            row8 == 7, 1.0, blk)
                        vt_win[kt, (hd + 1) * VR:(hd + 1) * VR + 8, :] = jnp.where(
                            row8 == 0, 1.0, blk)

        def oproj(slot, x_ref):
            hres_scr[slot] = x_ref[...].astype(f32) + jnp.dot(
                on_scr[...], wo_ref[...], preferred_element_type=f32)
            hn_scr[slot] = _layernorm_f32(hres_scr[slot]).astype(bf16)

        def ffn1(slot, r, c):
            rs = slice(r * FR, (r + 1) * FR)
            cs = slice(c * L, (c + F1) * L)
            a_scr[rs, cs] = jnp.maximum(
                jnp.dot(hn_scr[slot, rs, :], w1_ref[:, cs], preferred_element_type=f32),
                0.0).astype(bf16)

        def ffn2(slot, tile, early, r, c):
            rs = slice(r * FR, (r + 1) * FR)
            cs = slice(c * L, (c + 1) * L)
            y = hres_scr[slot, rs, cs] + jnp.dot(a_scr[rs, :], w2_ref[:, cs],
                                                 preferred_element_type=f32)
            o_win = o_scr.at[pl.ds(pl.multiple_of(tile * T, T), T)]
            o_win[rs, cs] = y.astype(bf16)
            if early and c == nd - 1:
                ocopy(tile * (T // FR) + r).start()

        def ffn_items(slot, tile, early=False):
            items = []
            for r in range(T // FR):
                items += [P(ffn1, slot, r, c) for c in range(0, Dff // L, F1)]
                items += [P(ffn2, slot, tile, early, r, c) for c in range(nd)]
            return items

        def cmin(t, b):
            return max(1, nc - t * QT // QB - b) if first else 1

        def scores(u):
            k_win, q_win = win[0], win[1]
            t, j = u // NG, u % NG
            hmask = []
            for i in range(G):
                l0 = ((j * G + i) * Dh) % L
                if l0 + Dh <= L:
                    hmask.append((lane >= l0) & (lane < l0 + Dh))
                else:
                    hmask.append((lane >= l0) | (lane < l0 + Dh - L))
            cs = slice(j * L, (j + 1) * L)
            ms = []
            for b in range(G):
                r0 = t * QT + b * QB
                qg = q_win[r0 // 2:(r0 + QB) // 2, cs]
                qm = _b16(jnp.concatenate(
                    [jnp.where(hmask[(c - b) % G], qg, jnp.uint32(0)) for c in range(G)],
                    axis=0))
                c1 = cmin(t, b)
                kparts = [k_win[r0 + W:r0 + W + QB, cs]]
                if c1 < nc:
                    kparts.append(k_win[r0 + c1 * QB:r0 + W, cs])
                if not first:
                    kparts.insert(0, k_win[r0:r0 + QB, cs])
                sc = lax.dot_general(jnp.concatenate(kparts, axis=0), qm, _NT,
                                     preferred_element_type=f32)
                if first:
                    parts = [jnp.where(tri, NEG, sc[0:QB])]
                    if c1 < nc:
                        parts.append(sc[QB:])
                else:
                    parts = [jnp.where(tri, sc[0:QB], sc[QB:2 * QB]), sc[2 * QB:]]
                sc = jnp.concatenate(parts, axis=0)
                s_scrs[(u % NB) * G + b][zw, 0:sc.shape[0]] = sc
                ms.append(jnp.max(sc, axis=0, keepdims=True))
                fence[u, b] = jnp.broadcast_to(ms[b], (8, QT))
            for b in range(G):
                i = (u % NB) * G + b
                rows = (nc - cmin(t, b) + 1) * QB
                p_scrs[i][zw, 0:rows // 2] = _pack16(
                    jnp.exp2(s_scrs[i][zr, 0:rows] - ms[b]))

        def pv(u):
            vt_win = win[3]
            t, j = u // NG, u % NG
            cols = slice(t * QT, (t + 1) * QT)
            p_scr = p_scrs[(u % NB) * G:(u % NB + 1) * G]
            fu = u + lag - 1
            if FENCE and fu < nu:
                for b in range(G):
                    p_scr[b][zw, W // 2:W // 2 + 8] = pltpu.bitcast(
                        fence[fu, b], jnp.uint32)

            def chunk(b, c):
                if c == nc:
                    pm = p_scr[b][zr, 0:hq]
                    return pm if first else pm & tri_c
                if c == 0 and not first:
                    return p_scr[b][zr, 0:hq] & tri_a
                c1 = cmin(t, b)
                if c < c1:
                    return None
                return p_scr[b][zr, (c - c1 + 1) * hq:(c - c1 + 2) * hq]

            def sel(msk, a, b):
                if a is None and b is None:
                    return None
                z = jnp.uint32(0)
                return jnp.where(msk, z if a is None else a, z if b is None else b)

            rows_per_head = [[] for _ in range(G)]
            for r in range(3 * QT // QB):
                xs = [chunk(b, r - b) if 0 <= r - b <= nc else None for b in range(G)]
                ys = [sel(bit0, xs[(m + 1) % G], xs[m]) for m in range(G)]
                zs = [sel(bit1, ys[(m + 2) % G], ys[m]) for m in range(G)]
                for i in range(G):
                    rows_per_head[i].append(zs[(-i) % G])

            os_ = [None] * G
            for c in range(2 - t if first else 0, 3):
                for i in range(G):
                    h = j * G + i
                    pc = _b16(jnp.concatenate(rows_per_head[i][c * G:(c + 1) * G], axis=0))
                    oc = jnp.dot(vt_win[t + c, h * VR:(h + 1) * VR, :], pc,
                                 preferred_element_type=f32)
                    os_[i] = oc if os_[i] is None else os_[i] + oc
            pend = None
            for i in range(G):
                c0 = (j * G + i) * Dh
                o = os_[i]
                r1 = 23 if c0 % 8 == 0 else 0
                o = o * (1.0 / o[r1:r1 + 1, :])
                if i:
                    o = pltpu.roll(o, QT - QB * i, 1)
                if c0 % 8 == 0:
                    ot_scr[c0:c0 + 16, cols] = o[0:16]
                    pend = o[16:24]
                else:
                    ot_scr[c0 - 4:c0 + 4, cols] = jnp.where(row8 < 4, pend, o[0:8])
                    ot_scr[c0 + 4:c0 + 20, cols] = o[8:24]
            if j == NG - 1:
                on_scr[cols, :] = ot_scr[:, cols].T.astype(bf16)

        def attention(items, tail, pos=None):
            done = 0
            tail = list(tail)
            for m in range(nu + lag):
                if m < nu:
                    scores(m)
                if m >= lag:
                    pv(m - lag)
                if m < nu:
                    want = ((m + 1) * len(items)) // nu
                    if pos is not None:
                        want = sum(p <= m for p in pos[:len(items)])
                    while done < want:
                        items[done]()
                        done += 1
                elif tail and m < nu + lag - 1:
                    tail.pop(0)()
            for it in tail:
                it()

        def seq(*fns):
            def run():
                for fn in fns:
                    fn()
            return run

        h = T // 2
        nr = T // FR
        xp_ref = x_scr.at[xrows(jnp.maximum(step - 1, 0))]
        xn_ref = x_scr.at[xrows(jnp.minimum(step + 1, n - 1))]
        if first:
            xcopy(0).start()
            for i in (0, 1, 2, 3, 4):
                wcopy(i).start()
            xcopy(1).start()
            for i in (5, 6):
                wcopy(i).start()
            xcopy(2).start()
            for i in (7, 8):
                wcopy(i).start()
            for i in range(3, n):
                xcopy(i).start()
            w0 = windows(zw)
            xcopy(0).wait()
            ln1(w0, 0, xp_ref)
            wcopy(0).wait()
            proj_qk(w0, 0, 0, T, 5, 9)
            wcopy(1).wait()
            wcopy(2).wait()
            proj_qk(w0, 0, 0, T, 9, 10)
            proj_qk(w0, 0, 0, T, 0, 3)
            wcopy(3).wait()
            wcopy(4).wait()
            proj_qk(w0, 0, 0, T, 3, 5)
            proj_v(w0, 0, 0, T, 0, 2)
            xcopy(1).wait()
            wcopy(5).wait()
            blocks.clear()
            ln1(win, T, xn_ref)
            items = [seq(P(proj_v, win, 0, 0, h, 2, 4), P(proj_v, win, 0, h, T, 2, 4)),
                     seq(P(proj_v, win, 0, 0, h, 4, 5), P(proj_v, win, 0, h, T, 4, 5),
                         P(proj_qk, win, T, 0, h, 0, 2)),
                     seq(P(proj_qk, win, T, h, T, 0, 2), P(proj_v, win, T, 0, h, 0, 2)),
                     P(proj_qk, win, T, 0, h, 2, 6), P(proj_qk, win, T, h, T, 2, 6),
                     seq(P(proj_v, win, T, h, T, 0, 2), P(proj_qk, win, T, 0, h, 6, 8)),
                     seq(P(proj_qk, win, T, 0, h, 8, 10), P(proj_qk, win, T, h, T, 6, 8)),
                     P(proj_qk, win, T, h, T, 8, 10)]
            attention(items[:len(items) - FT], items[len(items) - FT:], FPOS)
            for i in (6, 7, 8):
                wcopy(i).wait()
            xcopy(2).wait()
        elif not last:
            oproj(0, xp_ref)
            ln1(win, T, xn_ref)
            proj_v(win, 0, 0, T, 2, 5)
            attention(ffn_items(0, step - 1),
                      [seq(P(proj_v, win, T, 0, T, 0, 2), P(proj_qk, win, T, 0, T, 0, 2)),
                       P(proj_qk, win, T, 0, T, 2, 6), P(proj_qk, win, T, 0, T, 6, 10)])
            for r in range(nr):
                ocopy((step - 1) * nr + r).start()

            @pl.when(step + 2 < n)
            def _():
                xcopy(step + 2).wait()
        else:
            oproj(0, xp_ref)
            proj_v(win, 0, 0, T, 2, 5)
            items = ffn_items(0, n - 2)
            k = len(items) - LT1 - LT2
            attention(items[:k], items[k:k + LT1])
            oproj(1, xn_ref)
            for it in items[k + LT1:]:
                it()
            if EARLY:
                for r in range(nr):
                    ocopy((n - 2) * nr + r).start()
            for it in ffn_items(1, n - 1):
                it()
            for r in range(nr if EARLY else 0, 2 * nr):
                ocopy((n - 2) * nr + r).start()
            for i in range(n * nr):
                ocopy(i).wait()

    pl.when(step == 0)(P(body, True, False))
    pl.when((step > 0) & (step < n - 1))(P(body, False, False))
    pl.when(step == n - 1)(P(body, False, True))


@jax.jit
def pallas_sequential_preLN__sliding_block__dense_activation_relu__prompt_kernel(
    A_x: jax.Array,
    A_wqkv: jax.Array,
    A_wo: jax.Array,
    B_x: jax.Array,
    B_w1: jax.Array,
    B_w2: jax.Array,
):
    B, S, D = A_x.shape
    Dff = B_w1.shape[1]
    Dh = D // H
    assert B == 1 and S % T == 0 and S // T >= 3 and Dh == 20 and T == W
    n = S // T
    u32, f32 = jnp.uint32, jnp.float32

    hbm = pl.BlockSpec(memory_space=pl.ANY)
    out = pl.pallas_call(
        functools.partial(_kernel, D=D, Dh=Dh, Dff=Dff, n=n),
        grid=(n,),
        in_specs=[hbm] * 5,
        out_specs=hbm,
        out_shape=jax.ShapeDtypeStruct((B, S, D), A_x.dtype),
        scratch_shapes=[
            pltpu.VMEM((S // 2, D), u32),
            pltpu.VMEM((S // 2, D), u32),
            pltpu.VMEM((D // 2, 3 * D), u32),
            pltpu.VMEM((D // 2, D), u32),
            pltpu.VMEM((D // 2, Dff), u32),
            pltpu.VMEM((Dff // 2, D), u32),
            pltpu.VMEM(((S + W + T) // 2, NG * L), u32),
            pltpu.VMEM(((S + W + T) // QT, H * VR, QT), f32),
            pltpu.VMEM((D, T), f32),
            pltpu.VMEM((T // 2, D), u32),
            pltpu.VMEM((T // 2, D), u32),
            pltpu.VMEM(((S + T) // 2, D), u32),
            pltpu.VMEM(((S + T) // 2, NG * L), u32),
            pltpu.VMEM((2, T, D), f32),
            pltpu.VMEM((2, T // 2, D), u32),
            pltpu.VMEM((T // 2, Dff), u32),
            pltpu.SemaphoreType.DMA((9,)),
            pltpu.SemaphoreType.DMA((n,)),
            pltpu.SemaphoreType.DMA((S // FR,)),
        ] + [pltpu.VMEM((1, W, QT), f32)] * (NB * G)
          + [pltpu.VMEM((1, W // 2 + 8, QT), u32)] * (NB * G),
        compiler_params=pltpu.CompilerParams(
            dimension_semantics=("arbitrary",),
            vmem_limit_bytes=100 * 1024 * 1024,
        ),
        name="preln_swa_ffn",
    )(A_x, A_wqkv, A_wo, B_w1, B_w2)
    return out
```

```python
import functools
import math

import jax
import jax.numpy as jnp
from jax import lax
import jax.experimental.pallas as pl
import jax.experimental.pallas.tpu as pltpu

H = 32
W = 256
QT = 128
L = 128
EPS = 1e-5
NEG = -3.0e38
T = 256
G = 4
NG = H // G
VR = 24
QB = 32
FR = 128
F1 = 4
LAG = 3
NB = LAG + 1
LNQ = 4
FPOS = (0, 1, 2, 3, 4, 5, 6, 7, 11, 15)
SPOS = (1, 2, 3, 4, 5, 6, 7, 8, 9, 10, 11, 12, 13, 14, 15, 15)
LPOS = (0, 1, 2, 3, 4, 5, 6, 7, 8, 9, 10, 11, 12, 13, 14, 15, 15)

_NT = (((1,), (1,)), ((), ()))


def _layernorm_f32(x):
    m = jnp.mean(x, axis=-1, keepdims=True)
    xc = x - m
    v = jnp.mean(xc * xc, axis=-1, keepdims=True)
    return xc * lax.rsqrt(v + EPS)


def _b16(x):
    return pltpu.bitcast(x, jnp.bfloat16)


def _u32(x):
    return pltpu.bitcast(x, jnp.uint32)


def _kernel(x_hbm, wqkv_hbm, wo_hbm, w1_hbm, w2_hbm, o_hbm,
            x_scr, o_scr, wqkv_ref, wo_ref, w1_ref, w2_ref, k_scr, vt_scr, ot_scr,
            q_scr, hres_scr, hn_scr, act_scr, a_scr, sems, xsems, osems, *sp_scrs,
            D, Dh, Dff, n):
    step = pl.program_id(0)
    nq = T // QT
    npad = W // QT
    f32, bf16 = jnp.float32, jnp.bfloat16
    qscale = (Dh ** -0.5) * math.log2(math.e)
    hq = QB // 2
    nc = W // QB
    nd = D // L
    nu = nq * NG
    h = T // 2
    nr = T // FR
    P = functools.partial
    s_scrs = sp_scrs[:NB * G]
    zw = step // n
    zr = step // (n + 1)
    (x_scr, o_scr, wqkv_ref, wo_ref, w1_ref, w2_ref, k_scr, q_scr, hn_scr, act_scr,
     a_scr) = [r.bitcast(bf16) for r in
               (x_scr, o_scr, wqkv_ref, wo_ref, w1_ref, w2_ref, k_scr, q_scr, hn_scr,
                act_scr, a_scr)]
    p_scrs = [r.bitcast(bf16) for r in sp_scrs[NB * G:]]
    p_w = [r.at[pl.ds(zw, 1)].at[0] for r in p_scrs]
    p_r = [r.at[pl.ds(zr, 1)].at[0] for r in p_scrs]
    act_w = act_scr.at[pl.ds(zw, 3)]
    xn_scr, on_scr, xn0_scr = act_w.at[0], act_w.at[1], act_w.at[2]

    def xrows(i):
        return pl.ds(pl.multiple_of(i * T, T), T)

    def xt(i):
        return x_scr.at[xrows(i)]

    def xcopy(i):
        return pltpu.make_async_copy(x_hbm.at[0, xrows(i)], xt(i), xsems.at[i])

    def ocopy(i):
        rows = pl.ds(pl.multiple_of(i * FR, FR), FR)
        return pltpu.make_async_copy(o_scr.at[rows], o_hbm.at[0, rows], osems.at[i])

    qkv = lambda c0, c1: (wqkv_hbm, wqkv_ref, c0 * L, c1 * L)
    wlist = [qkv(5, 9), qkv(9, 10), qkv(0, 3), qkv(3, 5), qkv(10, 12), qkv(12, 15),
             (wo_hbm, wo_ref, 0, D), (w1_hbm, w1_ref, 0, Dff), (w2_hbm, w2_ref, 0, D)]

    def wcopy(i):
        src, dst, lo, hi = wlist[i]
        return pltpu.make_async_copy(src.at[:, lo:hi], dst.at[:, lo:hi], sems.at[i])

    def windows(tile):
        base = pl.multiple_of(tile * T, T)
        return (k_scr.at[pl.ds(base, W + 2 * T)],
                q_scr.at[pl.ds(base, 2 * T)],
                vt_scr.at[pl.ds(tile * nq, npad + 2 * nq)])

    def body(first, last):
        row8 = lax.broadcasted_iota(jnp.int32, (8, QT), 0)
        kk = lax.broadcasted_iota(jnp.int32, (QB, QT), 0)
        qq = lax.broadcasted_iota(jnp.int32, (QB, QT), 1) % QB
        tri = kk > qq
        lane = lax.broadcasted_iota(jnp.int32, (hq, QT), 1)
        k2 = 2 * lax.broadcasted_iota(jnp.int32, (hq, QT), 0)
        tri_a = (jnp.where(k2 > lane % QB, jnp.uint32(0xFFFF), jnp.uint32(0))
                 | jnp.where(k2 + 1 > lane % QB, jnp.uint32(0xFFFF0000), jnp.uint32(0)))
        tri_c = ~tri_a
        bit0 = (lane & QB) != 0
        bit1 = (lane & (2 * QB)) != 0
        tile0 = (0 if first else n - 1 if last else step) + zr
        win = windows(tile0)

        def ln1(dst, ref):
            deps = []
            for r0 in range(0, T, T // LNQ):
                r1 = r0 + T // LNQ
                xn32 = _layernorm_f32(ref[r0:r1, :].astype(f32))
                dst[r0:r1, :] = xn32.astype(bf16)
                d = _u32(xn32[0:8, D - L:D])
                for r in range(8, r1 - r0, 8):
                    d = d | _u32(xn32[r:r + 8, D - L:D])
                deps.append(d)
            return deps

        blocks = {}
        fence = {}

        def proj_qk(xn, w, po, r0, r1, c0, c1, cut=0):
            dot = P(jnp.dot, preferred_element_type=f32)
            if cut:
                e, q, cl = D - cut * L, (r1 - r0) // 4, slice((c1 - 1) * L, c1 * L)
                a = dot(xn[r0:r1, :], wqkv_ref[:, c0 * L:(c1 - 1) * L])
                a2 = dot(xn[r0:r1, 0:e], wqkv_ref[0:e, cl]) if e else None
                a3 = jnp.concatenate(
                    [dot(xn[r0 + i * q:r0 + (i + 1) * q, e:D], wqkv_ref[e:D, cl])
                     for i in range(4)], axis=0)
                a2 = a3 if a2 is None else a2 + a3
                a = jnp.concatenate([a, a2], axis=1)
            else:
                a = dot(xn[r0:r1, :], wqkv_ref[:, c0 * L:c1 * L])
            for c in range(c0, c1):
                blk = a[:, (c - c0) * L:(c - c0 + 1) * L]
                blocks[r0, c] = blk * qscale if c < nd else blk
            for j in range(2 * NG):
                f0 = (j % NG) * G * Dh
                g, l0 = f0 // L + (j // NG) * nd, f0 % L
                wrap = l0 + G * Dh > L
                if not c0 <= g + wrap < c1:
                    continue
                blk = blocks[r0, g]
                if wrap:
                    ln = lax.broadcasted_iota(jnp.int32, blk.shape, 1)
                    blk = jnp.where(ln >= l0, blk, blocks[r0, g + 1])
                js = slice((j % NG) * L, (j % NG + 1) * L)
                if j < NG:
                    w[1][po + r0:po + r1, js] = blk.astype(bf16)
                else:
                    w[0][W + po + r0:W + po + r1, js] = blk.astype(bf16)

        def proj_v(xn, w, po, r0, r1, c0, c1):
            vt_win = w[2]
            v = jnp.dot(xn[r0:r1, :], wqkv_ref[:, 2 * D + c0 * L:2 * D + c1 * L],
                        preferred_element_type=f32)
            for t in range(r0 // QT, r1 // QT):
                vt = v[t * QT - r0:(t + 1) * QT - r0, :].T
                kt = npad + po // QT + t
                for r in range((c1 - c0) * L // 8):
                    f0 = c0 * L + r * 8
                    blk = vt[r * 8:(r + 1) * 8]
                    hd = f0 // Dh
                    if (f0 + 7) // Dh == hd:
                        d0 = hd * VR + (f0 - hd * Dh + 4) // 8 * 8
                        vt_win[kt, d0:d0 + 8, :] = blk
                    else:
                        vt_win[kt, hd * VR + 16:hd * VR + 24, :] = jnp.where(
                            row8 == 7, 1.0, blk)
                        vt_win[kt, (hd + 1) * VR:(hd + 1) * VR + 8, :] = jnp.where(
                            row8 == 0, 1.0, blk)

        def oproj(slot, x_ref, r0, r1, deps=(), at=(2, 3, 4)):
            dot = P(jnp.dot, preferred_element_type=f32)
            deps = dict(zip(at, deps))

            def wo_blk(k1, c):
                cs = slice(c * L, (c + 1) * L)
                if c not in deps:
                    return wo_ref[0:k1, cs]
                head = _u32(wo_ref[0:16, cs]) | (deps[c] & zw.astype(jnp.uint32))
                return jnp.concatenate([_b16(head), wo_ref[16:k1, cs]], axis=0)

            e = D - L
            q = (r1 - r0) // 4
            o3 = jnp.concatenate(
                [dot(on_scr[r0 + i * q:r0 + (i + 1) * q, e:D], wo_ref[e:D, e:D])
                 for i in range(4)], axis=0)
            blks = [dot(on_scr[r0:r1, :], wo_blk(D, c)) for c in range(nd - 1)]
            o2 = dot(on_scr[r0:r1, 0:e], wo_blk(e, nd - 1)) + o3
            o = jnp.concatenate(blks + [o2], axis=1)
            hres_scr[slot, r0:r1] = x_ref[r0:r1, :].astype(f32) + o
            hn_scr[slot, r0:r1] = _layernorm_f32(hres_scr[slot, r0:r1]).astype(bf16)

        def ffn1(slot, r, c):
            rs = slice(r * FR, (r + 1) * FR)
            cs = slice(c * L, (c + F1) * L)
            a_scr[rs, cs] = jnp.maximum(
                jnp.dot(hn_scr[slot, rs, :], w1_ref[:, cs], preferred_element_type=f32),
                0.0).astype(bf16)

        def ffn2(slot, tile, r, c):
            rs = slice(r * FR, (r + 1) * FR)
            cs = slice(c * L, (c + 1) * L)
            y = hres_scr[slot, rs, cs] + jnp.dot(a_scr[rs, :], w2_ref[:, cs],
                                                 preferred_element_type=f32)
            o_scr.at[xrows(tile)][rs, cs] = y.astype(bf16)

        def ffn_items(slot, tile):
            items = []
            for r in range(nr):
                items += [P(ffn1, slot, r, c) for c in range(0, Dff // L, F1)]
                items += [P(ffn2, slot, tile, r, c) for c in range(nd)]
            return items

        def cmin(t, b):
            return max(1, nc - t * QT // QB - b) if first else 1

        def scores(u):
            k_win, q_win = win[0], win[1]
            t, j = u // NG, u % NG
            hmask = []
            for i in range(G):
                l0 = ((j * G + i) * Dh) % L
                if l0 + Dh <= L:
                    hmask.append((lane >= l0) & (lane < l0 + Dh))
                else:
                    hmask.append((lane >= l0) | (lane < l0 + Dh - L))
            cs = slice(j * L, (j + 1) * L)
            ms = []
            for b in range(G):
                r0 = t * QT + b * QB
                qg = _u32(q_win[r0:r0 + QB, cs])
                qm = _b16(jnp.concatenate(
                    [jnp.where(hmask[(c - b) % G], qg, jnp.uint32(0)) for c in range(G)],
                    axis=0))
                c1 = cmin(t, b)
                kparts = [k_win[r0 + W:r0 + W + QB, cs]]
                if c1 < nc:
                    kparts.append(k_win[r0 + c1 * QB:r0 + W, cs])
                if not first:
                    kparts.insert(0, k_win[r0:r0 + QB, cs])
                sc = lax.dot_general(jnp.concatenate(kparts, axis=0), qm, _NT,
                                     preferred_element_type=f32)
                if first:
                    parts = [jnp.where(tri, NEG, sc[0:QB])]
                    if c1 < nc:
                        parts.append(sc[QB:])
                else:
                    parts = [jnp.where(tri, sc[0:QB], sc[QB:2 * QB]), sc[2 * QB:]]
                sc = jnp.concatenate(parts, axis=0)
                s_scrs[(u % NB) * G + b][zw, 0:sc.shape[0]] = sc
                ms.append(jnp.max(sc, axis=0, keepdims=True))
                fence[u, b] = jnp.broadcast_to(ms[b], (8, QT))
            for b in range(G):
                i = (u % NB) * G + b
                rows = (nc - cmin(t, b) + 1) * QB
                p_w[u % NB][0:rows, b * L:(b + 1) * L] = jnp.exp2(
                    s_scrs[i][zr, 0:rows] - ms[b]).astype(bf16)

        def pv(u):
            vt_win = win[2]
            t, j = u // NG, u % NG
            cols = slice(t * QT, (t + 1) * QT)
            p_scr = [p_r[u % NB].at[:, b * L:(b + 1) * L] for b in range(G)]
            fu = u + LAG - 1
            if fu < nu:
                p_w[u % NB][W:W + 16, 0:L] = _b16(_u32(fence[fu, G - 1]))

            def chunk(b, c):
                if c == nc:
                    pm = _u32(p_scr[b][0:QB])
                    return pm if first else pm & tri_c
                if c == 0 and not first:
                    return _u32(p_scr[b][0:QB]) & tri_a
                c1 = cmin(t, b)
                if c < c1:
                    return None
                return _u32(p_scr[b][(c - c1 + 1) * QB:(c - c1 + 2) * QB])

            def sel(msk, a, b):
                if a is None and b is None:
                    return None
                z = jnp.uint32(0)
                return jnp.where(msk, z if a is None else a, z if b is None else b)

            rows_per_head = [[] for _ in range(G)]
            for r in range(3 * QT // QB):
                xs = [chunk(b, r - b) if 0 <= r - b <= nc else None for b in range(G)]
                ys = [sel(bit0, xs[(m + 1) % G], xs[m]) for m in range(G)]
                zs = [sel(bit1, ys[(m + 2) % G], ys[m]) for m in range(G)]
                for i in range(G):
                    rows_per_head[i].append(zs[(-i) % G])

            os_ = [None] * G
            for c in range(2 - t if first else 0, 3):
                for i in range(G):
                    hd = j * G + i
                    pc = _b16(jnp.concatenate(rows_per_head[i][c * G:(c + 1) * G], axis=0))
                    oc = jnp.dot(vt_win[t + c, hd * VR:(hd + 1) * VR, :], pc,
                                 preferred_element_type=f32)
                    os_[i] = oc if os_[i] is None else os_[i] + oc
            pend = None
            for i in range(G):
                c0 = (j * G + i) * Dh
                o = os_[i]
                r1 = 23 if c0 % 8 == 0 else 0
                o = o * (1.0 / o[r1:r1 + 1, :])
                if i:
                    o = pltpu.roll(o, QT - QB * i, 1)
                if c0 % 8 == 0:
                    ot_scr[c0:c0 + 16, cols] = o[0:16]
                    pend = o[16:24]
                else:
                    ot_scr[c0 - 4:c0 + 4, cols] = jnp.where(row8 < 4, pend, o[0:8])
                    ot_scr[c0 + 4:c0 + 20, cols] = o[8:24]
            if j == NG - 1:
                on_scr[cols, :] = ot_scr[:, cols].T.astype(bf16)

        def attention(items, pos, tail):
            assert len(items) == len(pos)
            done = 0
            tail = list(tail)
            for m in range(nu + LAG):
                if m < nu:
                    scores(m)
                if m >= LAG:
                    pv(m - LAG)
                if m < nu:
                    while done < len(items) and pos[done] <= m:
                        items[done]()
                        done += 1
                elif tail and m < nu + LAG - 1:
                    tail.pop(0)()
            for it in tail:
                it()

        def seq(*fns):
            def run():
                for fn in fns:
                    fn()
            return run

        V0 = lambda r0, r1, c0, c1: P(proj_v, xn0_scr, win, 0, r0, r1, c0, c1)
        V1 = lambda r0, r1, c0, c1: P(proj_v, xn_scr, win, T, r0, r1, c0, c1)
        QK = lambda *a: P(proj_qk, xn_scr, win, T, *a)
        if first:
            xcopy(0).start()
            for i in (0, 1, 2, 3, 4):
                wcopy(i).start()
            xcopy(1).start()
            for i in (5, 6):
                wcopy(i).start()
            xcopy(2).start()
            for i in (7, 8):
                wcopy(i).start()
            for i in range(3, n):
                xcopy(i).start()
            w0 = windows(zw)
            xcopy(0).wait()
            ln1(xn0_scr, xt(0))
            wcopy(0).wait()
            proj_qk(xn0_scr, w0, 0, 0, T, 5, 9)
            wcopy(1).wait()
            wcopy(2).wait()
            proj_qk(xn0_scr, w0, 0, 0, T, 9, 10)
            proj_qk(xn0_scr, w0, 0, 0, T, 0, 3)
            wcopy(3).wait()
            wcopy(4).wait()
            proj_v(xn0_scr, w0, 0, 0, T, 0, 2)
            proj_qk(xn0_scr, w0, 0, 0, T, 3, 5)
            xcopy(1).wait()
            wcopy(5).wait()
            blocks.clear()
            ln1(xn_scr, xt(1))
            attention([V0(0, h, 2, 4), V0(h, T, 2, 4), seq(V0(0, h, 4, 5), V0(h, T, 4, 5)),
                       QK(0, h, 0, 2), V1(0, h, 0, 2), V1(0, h, 2, 4), V1(h, T, 0, 2),
                       V1(h, T, 2, 4),
                       seq(V1(0, h, 4, 5), V1(h, T, 4, 5), QK(h, T, 0, 2)),
                       QK(0, h, 2, 6)], FPOS,
                      [QK(h, T, 2, 6), QK(0, h, 6, 10), QK(h, T, 6, 10)])
            for i in (6, 7, 8):
                wcopy(i).wait()
            xcopy(2).wait()
        elif not last:
            deps = ln1(xn_scr, xt(tile0 + 1))
            oproj(0, xt(tile0 - 1), 0, h, deps[:1], (3,))
            oproj(0, xt(tile0 - 1), h, T, deps[1:], (0, 2))
            attention(ffn_items(0, tile0 - 1), SPOS,
                      [V1(0, T, 0, 4), seq(V1(0, T, 4, 5), QK(0, T, 0, 3)),
                       QK(0, T, 3, 10, 4)])
            for r in range(nr):
                ocopy((tile0 - 1) * nr + r).start()

            @pl.when(tile0 + 2 < n)
            def _():
                xcopy(tile0 + 2).wait()
        else:
            oproj(0, xt(n - 2), 0, h)
            oproj(0, xt(n - 2), h, T)
            items = ffn_items(0, n - 2)
            items.insert(11, P(oproj, 1, xt(n - 1), 0, h))
            fin = ffn_items(1, n - 1)
            attention(items, LPOS, fin[:4])
            oproj(1, xt(n - 1), h, T)
            for it in fin[4:11]:
                it()
            for i in range((n - 2) * nr, n * nr - 1):
                ocopy(i).start()
            for it in fin[11:]:
                it()
            ocopy(n * nr - 1).start()
            for i in range(n * nr):
                ocopy(i).wait()

    pl.when(step == 0)(P(body, True, False))
    pl.when((step > 0) & (step < n - 1))(P(body, False, False))
    pl.when(step == n - 1)(P(body, False, True))


@jax.jit
def pallas_sequential_preLN__sliding_block__dense_activation_relu__prompt_kernel(
    A_x: jax.Array,
    A_wqkv: jax.Array,
    A_wo: jax.Array,
    B_x: jax.Array,
    B_w1: jax.Array,
    B_w2: jax.Array,
):
    B, S, D = A_x.shape
    Dff = B_w1.shape[1]
    Dh = D // H
    assert B == 1 and S % T == 0 and S // T >= 3 and T == W
    assert (D, Dh, Dff) == (640, 20, 1536)
    n = S // T
    u32, f32 = jnp.uint32, jnp.float32

    hbm = pl.BlockSpec(memory_space=pl.ANY)
    return pl.pallas_call(
        functools.partial(_kernel, D=D, Dh=Dh, Dff=Dff, n=n),
        grid=(n,),
        in_specs=[hbm] * 5,
        out_specs=hbm,
        out_shape=jax.ShapeDtypeStruct((B, S, D), A_x.dtype),
        scratch_shapes=[
            pltpu.VMEM((S // 2, D), u32),
            pltpu.VMEM((S // 2, D), u32),
            pltpu.VMEM((D // 2, 3 * D), u32),
            pltpu.VMEM((D // 2, D), u32),
            pltpu.VMEM((D // 2, Dff), u32),
            pltpu.VMEM((Dff // 2, D), u32),
            pltpu.VMEM(((S + W + T) // 2, NG * L), u32),
            pltpu.VMEM(((S + W + T) // QT, H * VR, QT), f32),
            pltpu.VMEM((D, T), f32),
            pltpu.VMEM(((S + T) // 2, NG * L), u32),
            pltpu.VMEM((2, T, D), f32),
            pltpu.VMEM((2, T // 2, D), u32),
            pltpu.VMEM((3, T // 2, D), u32),
            pltpu.VMEM((T // 2, Dff), u32),
            pltpu.SemaphoreType.DMA((9,)),
            pltpu.SemaphoreType.DMA((n,)),
            pltpu.SemaphoreType.DMA((S // FR,)),
        ] + [pltpu.VMEM((1, W, QT), f32)] * (NB * G)
          + [pltpu.VMEM((1, W // 2 + 8, G * QT), u32)] * NB,
        compiler_params=pltpu.CompilerParams(
            dimension_semantics=("arbitrary",),
            vmem_limit_bytes=100 * 1024 * 1024,
        ),
        name="preln_swa_ffn",
    )(A_x, A_wqkv, A_wo, B_w1, B_w2)
```

```python
import functools
import math

import jax
import jax.numpy as jnp
from jax import lax
import jax.experimental.pallas as pl
import jax.experimental.pallas.tpu as pltpu

H = 32
W = 256
QT = 128
L = 128
EPS = 1e-5
NEG = -3.0e38
T = 256
G = 4
NG = H // G
VR = 24
QB = 32
FR = 128
F1 = 4
LAG = 3
NB = LAG + 1
LNQ = 4
FPOS = (0, 1, 2, 3, 4, 5, 6, 7, 11, 15)
SPOS = (1, 2, 3, 4, 5, 6, 7, 8, 9, 10, 11, 12, 13, 14, 15, 15)
LPOS = (0, 1, 2, 3, 4, 5, 6, 7, 8, 9, 10, 11, 12, 13, 14, 15, 15)

_NT = (((1,), (1,)), ((), ()))


def _layernorm_f32(x):
    m = jnp.mean(x, axis=-1, keepdims=True)
    xc = x - m
    v = jnp.mean(xc * xc, axis=-1, keepdims=True)
    return xc * lax.rsqrt(v + EPS)


def _b16(x):
    return pltpu.bitcast(x, jnp.bfloat16)


def _u32(x):
    return pltpu.bitcast(x, jnp.uint32)


def _kernel(x_hbm, wqkv_hbm, wo_hbm, w1_hbm, w2_hbm, o_hbm,
            x_scr, o_scr, wqkv_ref, wo_ref, w1_ref, w2_ref, k_scr, vt_scr, ot_scr,
            q_scr, hres_scr, hn_scr, act_scr, a_scr, sems, xsems, osems, *sp_scrs,
            D, Dh, Dff, n):
    step = pl.program_id(0)
    nq = T // QT
    npad = W // QT
    f32, bf16 = jnp.float32, jnp.bfloat16
    qscale = (Dh ** -0.5) * math.log2(math.e)
    hq = QB // 2
    nc = W // QB
    nd = D // L
    nu = nq * NG
    h = T // 2
    nr = T // FR
    P = functools.partial
    s_scrs = sp_scrs[:NB * G]
    zw = lax.shift_right_logical(step, 16)
    zr = lax.shift_right_logical(step, 17)
    (x_scr, o_scr, wqkv_ref, wo_ref, w1_ref, w2_ref, k_scr, q_scr, hn_scr, act_scr,
     a_scr) = [r.bitcast(bf16) for r in
               (x_scr, o_scr, wqkv_ref, wo_ref, w1_ref, w2_ref, k_scr, q_scr, hn_scr,
                act_scr, a_scr)]
    p_scrs = [r.bitcast(bf16) for r in sp_scrs[NB * G:]]
    p_w = [r.at[pl.ds(zw, 1)].at[0] for r in p_scrs]
    p_r = [r.at[pl.ds(zr, 1)].at[0] for r in p_scrs]
    act_w = act_scr.at[pl.ds(zw, 3)]
    xn_scr, on_scr, xn0_scr = act_w.at[0], act_w.at[1], act_w.at[2]

    def xrows(i):
        return pl.ds(pl.multiple_of(i * T, T), T)

    def xt(i):
        return x_scr.at[xrows(i)]

    def xcopy(i):
        return pltpu.make_async_copy(x_hbm.at[0, xrows(i)], xt(i), xsems.at[i])

    def ocopy(i):
        if isinstance(i, int) and i >= n - 2:
            lo = (n - 2) * T if i == n - 2 else n * T - FR
            hi = n * T - FR if i == n - 2 else n * T
            rows = pl.ds(lo, hi - lo)
        else:
            rows = xrows(i)
        return pltpu.make_async_copy(o_scr.at[rows], o_hbm.at[0, rows], osems.at[i])

    qkv = lambda c0, c1: (wqkv_hbm, wqkv_ref, c0 * L, c1 * L)
    wlist = [qkv(5, 9), qkv(9, 10), qkv(0, 3), qkv(3, 5), qkv(10, 12), qkv(12, 15),
             (wo_hbm, wo_ref, 0, D), (w1_hbm, w1_ref, 0, Dff), (w2_hbm, w2_ref, 0, D)]

    def wcopy(i):
        src, dst, lo, hi = wlist[i]
        return pltpu.make_async_copy(src.at[:, lo:hi], dst.at[:, lo:hi], sems.at[i])

    def windows(tile):
        base = pl.multiple_of(tile * T, T)
        return (k_scr.at[pl.ds(base, W + 2 * T)],
                q_scr.at[pl.ds(base, 2 * T)],
                vt_scr.at[pl.ds(tile * nq, npad + 2 * nq)])

    def body(first, last):
        row8 = lax.broadcasted_iota(jnp.int32, (8, QT), 0)
        kk = lax.broadcasted_iota(jnp.int32, (QB, QT), 0)
        qq = lax.broadcasted_iota(jnp.int32, (QB, QT), 1) % QB
        tri = kk > qq
        lane = lax.broadcasted_iota(jnp.int32, (hq, QT), 1)
        k2 = 2 * lax.broadcasted_iota(jnp.int32, (hq, QT), 0)
        tri_a = (jnp.where(k2 > lane % QB, jnp.uint32(0xFFFF), jnp.uint32(0))
                 | jnp.where(k2 + 1 > lane % QB, jnp.uint32(0xFFFF0000), jnp.uint32(0)))
        tri_c = ~tri_a
        bit0 = (lane & QB) != 0
        bit1 = (lane & (2 * QB)) != 0
        tile0 = (0 if first else n - 1 if last else step) + zr
        win = windows(tile0)

        def ln1(dst, ref):
            deps = []
            for r0 in range(0, T, T // LNQ):
                r1 = r0 + T // LNQ
                xn32 = _layernorm_f32(ref[r0:r1, :].astype(f32))
                dst[r0:r1, :] = xn32.astype(bf16)
                d = _u32(xn32[0:8, D - L:D])
                for r in range(8, r1 - r0, 8):
                    d = d | _u32(xn32[r:r + 8, D - L:D])
                deps.append(d)
            return deps

        blocks = {}
        fence = {}

        def proj_qk(xn, w, po, r0, r1, c0, c1, cut=0):
            dot = P(jnp.dot, preferred_element_type=f32)
            if cut:
                e, q, cl = D - cut * L, (r1 - r0) // 4, slice((c1 - 1) * L, c1 * L)
                a = dot(xn[r0:r1, :], wqkv_ref[:, c0 * L:(c1 - 1) * L])
                a2 = dot(xn[r0:r1, 0:e], wqkv_ref[0:e, cl]) if e else None
                a3 = jnp.concatenate(
                    [dot(xn[r0 + i * q:r0 + (i + 1) * q, e:D], wqkv_ref[e:D, cl])
                     for i in range(4)], axis=0)
                a2 = a3 if a2 is None else a2 + a3
                a = jnp.concatenate([a, a2], axis=1)
            else:
                a = dot(xn[r0:r1, :], wqkv_ref[:, c0 * L:c1 * L])
            for c in range(c0, c1):
                blk = a[:, (c - c0) * L:(c - c0 + 1) * L]
                blocks[r0, c] = blk * qscale if c < nd else blk
            for j in range(2 * NG):
                f0 = (j % NG) * G * Dh
                g, l0 = f0 // L + (j // NG) * nd, f0 % L
                wrap = l0 + G * Dh > L
                if not c0 <= g + wrap < c1:
                    continue
                blk = blocks[r0, g]
                if wrap:
                    ln = lax.broadcasted_iota(jnp.int32, blk.shape, 1)
                    blk = jnp.where(ln >= l0, blk, blocks[r0, g + 1])
                js = slice((j % NG) * L, (j % NG + 1) * L)
                if j < NG:
                    w[1][po + r0:po + r1, js] = blk.astype(bf16)
                else:
                    w[0][W + po + r0:W + po + r1, js] = blk.astype(bf16)

        def proj_v(xn, w, po, r0, r1, c0, c1):
            vt_win = w[2]
            v = jnp.dot(xn[r0:r1, :], wqkv_ref[:, 2 * D + c0 * L:2 * D + c1 * L],
                        preferred_element_type=f32)
            for t in range(r0 // QT, r1 // QT):
                vt = v[t * QT - r0:(t + 1) * QT - r0, :].T
                kt = npad + po // QT + t
                for r in range((c1 - c0) * L // 8):
                    f0 = c0 * L + r * 8
                    blk = vt[r * 8:(r + 1) * 8]
                    hd = f0 // Dh
                    if (f0 + 7) // Dh == hd:
                        d0 = hd * VR + (f0 - hd * Dh + 4) // 8 * 8
                        vt_win[kt, d0:d0 + 8, :] = blk
                    else:
                        vt_win[kt, hd * VR + 16:hd * VR + 24, :] = jnp.where(
                            row8 == 7, 1.0, blk)
                        vt_win[kt, (hd + 1) * VR:(hd + 1) * VR + 8, :] = jnp.where(
                            row8 == 0, 1.0, blk)

        def oproj(slot, x_ref, r0, r1, deps=(), at=(2, 3, 4)):
            dot = P(jnp.dot, preferred_element_type=f32)
            deps = dict(zip(at, deps))

            def wo_blk(k1, c):
                cs = slice(c * L, (c + 1) * L)
                if c not in deps:
                    return wo_ref[0:k1, cs]
                head = _u32(wo_ref[0:16, cs]) | (deps[c] & zw.astype(jnp.uint32))
                return jnp.concatenate([_b16(head), wo_ref[16:k1, cs]], axis=0)

            e = D - L
            q = (r1 - r0) // 4
            o3 = jnp.concatenate(
                [dot(on_scr[r0 + i * q:r0 + (i + 1) * q, e:D], wo_ref[e:D, e:D])
                 for i in range(4)], axis=0)
            blks = [dot(on_scr[r0:r1, :], wo_blk(D, c)) for c in range(nd - 1)]
            o2 = dot(on_scr[r0:r1, 0:e], wo_blk(e, nd - 1)) + o3
            o = jnp.concatenate(blks + [o2], axis=1)
            hres_scr[slot, r0:r1] = x_ref[r0:r1, :].astype(f32) + o
            hn_scr[slot, r0:r1] = _layernorm_f32(hres_scr[slot, r0:r1]).astype(bf16)

        def ffn1(slot, r, c):
            rs = slice(r * FR, (r + 1) * FR)
            cs = slice(c * L, (c + F1) * L)
            a_scr[rs, cs] = jnp.maximum(
                jnp.dot(hn_scr[slot, rs, :], w1_ref[:, cs], preferred_element_type=f32),
                0.0).astype(bf16)

        def ffn2(slot, tile, r, c):
            rs = slice(r * FR, (r + 1) * FR)
            cs = slice(c * L, (c + 1) * L)
            y = hres_scr[slot, rs, cs] + jnp.dot(a_scr[rs, :], w2_ref[:, cs],
                                                 preferred_element_type=f32)
            o_scr.at[xrows(tile)][rs, cs] = y.astype(bf16)

        def ffn_items(slot, tile):
            items = []
            for r in range(nr):
                items += [P(ffn1, slot, r, c) for c in range(0, Dff // L, F1)]
                items += [P(ffn2, slot, tile, r, c) for c in range(nd)]
            return items

        def cmin(t, b):
            return max(1, nc - t * QT // QB - b) if first else 1

        def scores(u):
            k_win, q_win = win[0], win[1]
            t, j = u // NG, u % NG
            hmask = []
            for i in range(G):
                l0 = ((j * G + i) * Dh) % L
                if l0 + Dh <= L:
                    hmask.append((lane >= l0) & (lane < l0 + Dh))
                else:
                    hmask.append((lane >= l0) | (lane < l0 + Dh - L))
            cs = slice(j * L, (j + 1) * L)
            ms = []
            for b in range(G):
                r0 = t * QT + b * QB
                qg = _u32(q_win[r0:r0 + QB, cs])
                qm = _b16(jnp.concatenate(
                    [jnp.where(hmask[(c - b) % G], qg, jnp.uint32(0)) for c in range(G)],
                    axis=0))
                c1 = cmin(t, b)
                kparts = [k_win[r0 + W:r0 + W + QB, cs]]
                if c1 < nc:
                    kparts.append(k_win[r0 + c1 * QB:r0 + W, cs])
                if not first:
                    kparts.insert(0, k_win[r0:r0 + QB, cs])
                sc = lax.dot_general(jnp.concatenate(kparts, axis=0), qm, _NT,
                                     preferred_element_type=f32)
                if first:
                    parts = [jnp.where(tri, NEG, sc[0:QB])]
                    if c1 < nc:
                        parts.append(sc[QB:])
                else:
                    parts = [jnp.where(tri, sc[0:QB], sc[QB:2 * QB]), sc[2 * QB:]]
                sc = jnp.concatenate(parts, axis=0)
                s_scrs[(u % NB) * G + b][zw, 0:sc.shape[0]] = sc
                ms.append(jnp.max(sc, axis=0, keepdims=True))
                fence[u, b] = jnp.broadcast_to(ms[b], (8, QT))
            for b in range(G):
                i = (u % NB) * G + b
                rows = (nc - cmin(t, b) + 1) * QB
                p_w[u % NB][0:rows, b * L:(b + 1) * L] = jnp.exp2(
                    s_scrs[i][zr, 0:rows] - ms[b]).astype(bf16)

        def pv(u):
            vt_win = win[2]
            t, j = u // NG, u % NG
            cols = slice(t * QT, (t + 1) * QT)
            p_scr = [p_r[u % NB].at[:, b * L:(b + 1) * L] for b in range(G)]
            fu = u + LAG - 1
            if fu < nu:
                p_w[u % NB][W:W + 16, 0:L] = _b16(_u32(fence[fu, G - 1]))

            def chunk(b, c):
                if c == nc:
                    pm = _u32(p_scr[b][0:QB])
                    return pm if first else pm & tri_c
                if c == 0 and not first:
                    return _u32(p_scr[b][0:QB]) & tri_a
                c1 = cmin(t, b)
                if c < c1:
                    return None
                return _u32(p_scr[b][(c - c1 + 1) * QB:(c - c1 + 2) * QB])

            def sel(msk, a, b):
                if a is None and b is None:
                    return None
                z = jnp.uint32(0)
                return jnp.where(msk, z if a is None else a, z if b is None else b)

            rows_per_head = [[] for _ in range(G)]
            for r in range(3 * QT // QB):
                xs = [chunk(b, r - b) if 0 <= r - b <= nc else None for b in range(G)]
                ys = [sel(bit0, xs[(m + 1) % G], xs[m]) for m in range(G)]
                zs = [sel(bit1, ys[(m + 2) % G], ys[m]) for m in range(G)]
                for i in range(G):
                    rows_per_head[i].append(zs[(-i) % G])

            os_ = [None] * G
            for c in range(2 - t if first else 0, 3):
                for i in range(G):
                    hd = j * G + i
                    pc = _b16(jnp.concatenate(rows_per_head[i][c * G:(c + 1) * G], axis=0))
                    oc = jnp.dot(vt_win[t + c, hd * VR:(hd + 1) * VR, :], pc,
                                 precision=lax.Precision.DEFAULT,
                                 preferred_element_type=f32)
                    os_[i] = oc if os_[i] is None else os_[i] + oc
            pend = None
            for i in range(G):
                c0 = (j * G + i) * Dh
                o = os_[i]
                r1 = 23 if c0 % 8 == 0 else 0
                o = o * (1.0 / o[r1:r1 + 1, :])
                if i:
                    o = pltpu.roll(o, QT - QB * i, 1)
                if c0 % 8 == 0:
                    ot_scr[c0:c0 + 16, cols] = o[0:16]
                    pend = o[16:24]
                else:
                    ot_scr[c0 - 4:c0 + 4, cols] = jnp.where(row8 < 4, pend, o[0:8])
                    ot_scr[c0 + 4:c0 + 20, cols] = o[8:24]
            if j == NG - 1:
                on_scr[cols, :] = ot_scr[:, cols].T.astype(bf16)

        def attention(items, pos, tail):
            assert len(items) == len(pos)
            done = 0
            tail = list(tail)
            for m in range(nu + LAG):
                if m < nu:
                    scores(m)
                if m >= LAG:
                    pv(m - LAG)
                if m < nu:
                    while done < len(items) and pos[done] <= m:
                        items[done]()
                        done += 1
                elif tail and m < nu + LAG - 1:
                    tail.pop(0)()
            for it in tail:
                it()

        def seq(*fns):
            def run():
                for fn in fns:
                    fn()
            return run

        V0 = lambda r0, r1, c0, c1: P(proj_v, xn0_scr, win, 0, r0, r1, c0, c1)
        V1 = lambda r0, r1, c0, c1: P(proj_v, xn_scr, win, T, r0, r1, c0, c1)
        QK = lambda *a: P(proj_qk, xn_scr, win, T, *a)
        if first:
            xcopy(0).start()
            for i in (0, 1, 2, 3, 4):
                wcopy(i).start()
            xcopy(1).start()
            for i in (5, 6):
                wcopy(i).start()
            xcopy(2).start()
            for i in (7, 8):
                wcopy(i).start()
            for i in range(3, n):
                xcopy(i).start()
            w0 = windows(zw)
            xcopy(0).wait()
            ln1(xn0_scr, xt(0))
            wcopy(0).wait()
            proj_qk(xn0_scr, w0, 0, 0, T, 5, 9)
            wcopy(1).wait()
            wcopy(2).wait()
            proj_qk(xn0_scr, w0, 0, 0, T, 9, 10)
            proj_qk(xn0_scr, w0, 0, 0, T, 0, 3)
            wcopy(3).wait()
            wcopy(4).wait()
            proj_v(xn0_scr, w0, 0, 0, T, 0, 2)
            proj_qk(xn0_scr, w0, 0, 0, T, 3, 5)
            xcopy(1).wait()
            wcopy(5).wait()
            blocks.clear()
            ln1(xn_scr, xt(1))
            attention([V0(0, h, 2, 4), V0(h, T, 2, 4), seq(V0(0, h, 4, 5), V0(h, T, 4, 5)),
                       QK(0, h, 0, 2), V1(0, h, 0, 2), V1(0, h, 2, 4), V1(h, T, 0, 2),
                       V1(h, T, 2, 4),
                       seq(V1(0, h, 4, 5), V1(h, T, 4, 5), QK(h, T, 0, 2)),
                       QK(0, h, 2, 6)], FPOS,
                      [QK(h, T, 2, 6), QK(0, h, 6, 10), QK(h, T, 6, 10)])
            for i in (6, 7, 8):
                wcopy(i).wait()
            xcopy(2).wait()
        elif not last:
            deps = ln1(xn_scr, xt(tile0 + 1))
            oproj(0, xt(tile0 - 1), 0, h, deps[:1], (3,))
            oproj(0, xt(tile0 - 1), h, T, deps[1:], (0, 2))
            attention(ffn_items(0, tile0 - 1), SPOS,
                      [V1(0, T, 0, 4), seq(V1(0, T, 4, 5), QK(0, T, 0, 3)),
                       QK(0, T, 3, 10, 4)])
            ocopy(tile0 - 1).start()

            @pl.when(tile0 + 2 < n)
            def _():
                xcopy(tile0 + 2).wait()
        else:
            oproj(0, xt(n - 2), 0, h)
            oproj(0, xt(n - 2), h, T)
            items = ffn_items(0, n - 2)
            items.insert(11, P(oproj, 1, xt(n - 1), 0, h))
            fin = ffn_items(1, n - 1)
            attention(items, LPOS, fin[:4])
            oproj(1, xt(n - 1), h, T)
            for it in fin[4:11]:
                it()
            ocopy(n - 2).start()
            for it in fin[11:]:
                it()
            ocopy(n - 1).start()
            for i in range(n):
                ocopy(i).wait()

    lax.cond((step > 0) & (step < n - 1), P(body, False, False),
             lambda: lax.cond(step == 0, P(body, True, False), P(body, False, True)))


@jax.jit
def pallas_sequential_preLN__sliding_block__dense_activation_relu__prompt_kernel(
    A_x: jax.Array,
    A_wqkv: jax.Array,
    A_wo: jax.Array,
    B_x: jax.Array,
    B_w1: jax.Array,
    B_w2: jax.Array,
):
    B, S, D = A_x.shape
    Dff = B_w1.shape[1]
    Dh = D // H
    assert B == 1 and S % T == 0 and S // T >= 3 and T == W
    assert (D, Dh, Dff) == (640, 20, 1536)
    n = S // T
    u32, f32 = jnp.uint32, jnp.float32

    hbm = pl.BlockSpec(memory_space=pl.ANY)
    return pl.pallas_call(
        functools.partial(_kernel, D=D, Dh=Dh, Dff=Dff, n=n),
        grid=(n,),
        in_specs=[hbm] * 5,
        out_specs=hbm,
        out_shape=jax.ShapeDtypeStruct((B, S, D), A_x.dtype),
        scratch_shapes=[
            pltpu.VMEM((S // 2, D), u32),
            pltpu.VMEM((S // 2, D), u32),
            pltpu.VMEM((D // 2, 3 * D), u32),
            pltpu.VMEM((D // 2, D), u32),
            pltpu.VMEM((D // 2, Dff), u32),
            pltpu.VMEM((Dff // 2, D), u32),
            pltpu.VMEM(((S + W + T) // 2, NG * L), u32),
            pltpu.VMEM(((S + W + T) // QT, H * VR, QT), f32),
            pltpu.VMEM((D, T), f32),
            pltpu.VMEM(((S + T) // 2, NG * L), u32),
            pltpu.VMEM((2, T, D), f32),
            pltpu.VMEM((2, T // 2, D), u32),
            pltpu.VMEM((3, T // 2, D), u32),
            pltpu.VMEM((T // 2, Dff), u32),
            pltpu.SemaphoreType.DMA((9,)),
            pltpu.SemaphoreType.DMA((n,)),
            pltpu.SemaphoreType.DMA((n,)),
        ] + [pltpu.VMEM((1, W, QT), f32)] * (NB * G)
          + [pltpu.VMEM((1, W // 2 + 8, G * QT), u32)] * NB,
        compiler_params=pltpu.CompilerParams(
            dimension_semantics=("arbitrary",),
            vmem_limit_bytes=100 * 1024 * 1024,
        ),
        name="preln_swa_ffn",
    )(A_x, A_wqkv, A_wo, B_w1, B_w2)
```

```python
import functools
import math

import jax
import jax.numpy as jnp
from jax import lax
import jax.experimental.pallas as pl
import jax.experimental.pallas.tpu as pltpu

H = 32
W = 256
QT = 128
L = 128
EPS = 1e-5
NEG = -3.0e38
T = 256
G = 4
NG = H // G
VR = 24
QB = 32
FR = 128
F1 = 4
LAG = 3
NB = LAG + 1
LNQ = 4
FPOS = (0, 1, 2, 3, 4, 5, 6, 7, 11, 15)
SPOS = (1, 2, 3, 4, 5, 6, 7, 8, 9, 10, 11, 12, 13, 14, 15, 15)
LPOS = (0, 1, 2, 3, 4, 5, 6, 7, 8, 9, 10, 11, 12, 13, 14, 15, 15)

_NT = (((1,), (1,)), ((), ()))


def _layernorm_f32(x):
    m = jnp.mean(x, axis=-1, keepdims=True)
    xc = x - m
    v = jnp.mean(xc * xc, axis=-1, keepdims=True)
    return xc * lax.rsqrt(v + EPS)


def _b16(x):
    return pltpu.bitcast(x, jnp.bfloat16)


def _u32(x):
    return pltpu.bitcast(x, jnp.uint32)


def _kernel(x_hbm, wqkv_hbm, wo_hbm, w1_hbm, w2_hbm, o_hbm,
            x_scr, o_scr, wqkv_ref, wo_ref, w1_ref, w2_ref, k_scr, vt_scr, ot_scr,
            q_scr, hres_scr, hn_scr, act_scr, a_scr, sems, xsems, osems, *sp_scrs,
            D, Dh, Dff, n):
    step = pl.program_id(0)
    nq = T // QT
    npad = W // QT
    f32, bf16 = jnp.float32, jnp.bfloat16
    qscale = (Dh ** -0.5) * math.log2(math.e)
    hq = QB // 2
    nc = W // QB
    nd = D // L
    nu = nq * NG
    h = T // 2
    nr = T // FR
    P = functools.partial
    s_scrs = sp_scrs[:NB * G]
    zw = lax.shift_right_logical(step, 16)
    zr = lax.shift_right_logical(step, 17)
    (x_scr, o_scr, wqkv_ref, wo_ref, w1_ref, w2_ref, k_scr, q_scr, hn_scr, act_scr,
     a_scr) = [r.bitcast(bf16) for r in
               (x_scr, o_scr, wqkv_ref, wo_ref, w1_ref, w2_ref, k_scr, q_scr, hn_scr,
                act_scr, a_scr)]
    p_scrs = [r.bitcast(bf16) for r in sp_scrs[NB * G:]]
    p_w = [r.at[pl.ds(zw, 1)].at[0] for r in p_scrs]
    p_r = [r.at[pl.ds(zr, 1)].at[0] for r in p_scrs]
    act_w = act_scr.at[pl.ds(zw, 3)]
    xn_scr, on_scr, xn0_scr = act_w.at[0], act_w.at[1], act_w.at[2]

    def xrows(i):
        return pl.ds(pl.multiple_of(i * T, T), T)

    def xt(i):
        return x_scr.at[xrows(i)]

    def xcopy(i):
        return pltpu.make_async_copy(x_hbm.at[0, xrows(i)], xt(i), xsems.at[i])

    def ocopy(i):
        if isinstance(i, int) and i >= n - 2:
            lo = (n - 2) * T if i == n - 2 else n * T - FR
            hi = n * T - FR if i == n - 2 else n * T
            rows = pl.ds(lo, hi - lo)
        else:
            rows = xrows(i)
        return pltpu.make_async_copy(o_scr.at[rows], o_hbm.at[0, rows], osems.at[i])

    qkv = lambda c0, c1: (wqkv_hbm, wqkv_ref, c0 * L, c1 * L)
    wlist = [qkv(0, 4), qkv(4, 8), qkv(8, 12), qkv(12, 15),
             (wo_hbm, wo_ref, 0, D), (w1_hbm, w1_ref, 0, Dff), (w2_hbm, w2_ref, 0, D)]

    def wcopy(i):
        src, dst, lo, hi = wlist[i]
        return pltpu.make_async_copy(src.at[:, lo:hi], dst.at[:, lo:hi], sems.at[i])

    def windows(tile):
        base = pl.multiple_of(tile * T, T)
        return (k_scr.at[pl.ds(base, W + 2 * T)],
                q_scr.at[pl.ds(base, 2 * T)],
                vt_scr.at[pl.ds(tile * nq, npad + 2 * nq)])

    def body(first, last):
        row8 = lax.broadcasted_iota(jnp.int32, (8, QT), 0)
        kk = lax.broadcasted_iota(jnp.int32, (QB, QT), 0)
        qq = lax.broadcasted_iota(jnp.int32, (QB, QT), 1) % QB
        tri = kk > qq
        lane = lax.broadcasted_iota(jnp.int32, (hq, QT), 1)
        k2 = 2 * lax.broadcasted_iota(jnp.int32, (hq, QT), 0)
        tri_a = (jnp.where(k2 > lane % QB, jnp.uint32(0xFFFF), jnp.uint32(0))
                 | jnp.where(k2 + 1 > lane % QB, jnp.uint32(0xFFFF0000), jnp.uint32(0)))
        tri_c = ~tri_a
        bit0 = (lane & QB) != 0
        bit1 = (lane & (2 * QB)) != 0
        tile0 = (0 if first else n - 1 if last else step) + zr
        win = windows(tile0)

        def ln1(dst, ref):
            deps = []
            for r0 in range(0, T, T // LNQ):
                r1 = r0 + T // LNQ
                xn32 = _layernorm_f32(ref[r0:r1, :].astype(f32))
                dst[r0:r1, :] = xn32.astype(bf16)
                d = _u32(xn32[0:8, D - L:D])
                for r in range(8, r1 - r0, 8):
                    d = d | _u32(xn32[r:r + 8, D - L:D])
                deps.append(d)
            return deps

        blocks = {}
        fence = {}

        def proj_qk(xn, w, po, r0, r1, c0, c1, cut=0):
            dot = P(jnp.dot, preferred_element_type=f32)
            if cut:
                e, q, cl = D - cut * L, (r1 - r0) // 4, slice((c1 - 1) * L, c1 * L)
                a = dot(xn[r0:r1, :], wqkv_ref[:, c0 * L:(c1 - 1) * L])
                a2 = dot(xn[r0:r1, 0:e], wqkv_ref[0:e, cl]) if e else None
                a3 = jnp.concatenate(
                    [dot(xn[r0 + i * q:r0 + (i + 1) * q, e:D], wqkv_ref[e:D, cl])
                     for i in range(4)], axis=0)
                a2 = a3 if a2 is None else a2 + a3
                a = jnp.concatenate([a, a2], axis=1)
            else:
                a = dot(xn[r0:r1, :], wqkv_ref[:, c0 * L:c1 * L])
            for c in range(c0, c1):
                blk = a[:, (c - c0) * L:(c - c0 + 1) * L]
                blocks[r0, c] = blk * qscale if c < nd else blk
            for j in range(2 * NG):
                f0 = (j % NG) * G * Dh
                g, l0 = f0 // L + (j // NG) * nd, f0 % L
                wrap = l0 + G * Dh > L
                if not c0 <= g + wrap < c1:
                    continue
                blk = blocks[r0, g]
                if wrap:
                    ln = lax.broadcasted_iota(jnp.int32, blk.shape, 1)
                    blk = jnp.where(ln >= l0, blk, blocks[r0, g + 1])
                js = slice((j % NG) * L, (j % NG + 1) * L)
                if j < NG:
                    w[1][po + r0:po + r1, js] = blk.astype(bf16)
                else:
                    w[0][W + po + r0:W + po + r1, js] = blk.astype(bf16)

        def proj_v(xn, w, po, r0, r1, c0, c1):
            vt_win = w[2]
            v = jnp.dot(xn[r0:r1, :], wqkv_ref[:, 2 * D + c0 * L:2 * D + c1 * L],
                        preferred_element_type=f32)
            for t in range(r0 // QT, r1 // QT):
                vt = v[t * QT - r0:(t + 1) * QT - r0, :].T
                kt = npad + po // QT + t
                for r in range((c1 - c0) * L // 8):
                    f0 = c0 * L + r * 8
                    blk = vt[r * 8:(r + 1) * 8]
                    hd = f0 // Dh
                    if (f0 + 7) // Dh == hd:
                        d0 = hd * VR + (f0 - hd * Dh + 4) // 8 * 8
                        vt_win[kt, d0:d0 + 8, :] = blk
                    else:
                        vt_win[kt, hd * VR + 16:hd * VR + 24, :] = jnp.where(
                            row8 == 7, 1.0, blk)
                        vt_win[kt, (hd + 1) * VR:(hd + 1) * VR + 8, :] = jnp.where(
                            row8 == 0, 1.0, blk)

        def oproj(slot, x_ref, r0, r1, deps=(), at=(2, 3, 4)):
            dot = P(jnp.dot, preferred_element_type=f32)
            deps = dict(zip(at, deps))

            def wo_blk(k1, c):
                cs = slice(c * L, (c + 1) * L)
                if c not in deps:
                    return wo_ref[0:k1, cs]
                head = _u32(wo_ref[0:16, cs]) | (deps[c] & zw.astype(jnp.uint32))
                return jnp.concatenate([_b16(head), wo_ref[16:k1, cs]], axis=0)

            e = D - L
            q = (r1 - r0) // 4
            o3 = jnp.concatenate(
                [dot(on_scr[r0 + i * q:r0 + (i + 1) * q, e:D], wo_ref[e:D, e:D])
                 for i in range(4)], axis=0)
            blks = [dot(on_scr[r0:r1, :], wo_blk(D, c)) for c in range(nd - 1)]
            o2 = dot(on_scr[r0:r1, 0:e], wo_blk(e, nd - 1)) + o3
            o = jnp.concatenate(blks + [o2], axis=1)
            hres_scr[slot, r0:r1] = x_ref[r0:r1, :].astype(f32) + o
            hn_scr[slot, r0:r1] = _layernorm_f32(hres_scr[slot, r0:r1]).astype(bf16)

        def ffn1(slot, r, c):
            rs = slice(r * FR, (r + 1) * FR)
            cs = slice(c * L, (c + F1) * L)
            a_scr[rs, cs] = jnp.maximum(
                jnp.dot(hn_scr[slot, rs, :], w1_ref[:, cs], preferred_element_type=f32),
                0.0).astype(bf16)

        def ffn2(slot, tile, r, c):
            rs = slice(r * FR, (r + 1) * FR)
            cs = slice(c * L, (c + 1) * L)
            y = hres_scr[slot, rs, cs] + jnp.dot(a_scr[rs, :], w2_ref[:, cs],
                                                 preferred_element_type=f32)
            o_scr.at[xrows(tile)][rs, cs] = y.astype(bf16)

        def ffn_items(slot, tile):
            items = []
            for r in range(nr):
                items += [P(ffn1, slot, r, c) for c in range(0, Dff // L, F1)]
                items += [P(ffn2, slot, tile, r, c) for c in range(nd)]
            return items

        def cmin(t, b):
            return max(1, nc - t * QT // QB - b) if first else 1

        def scores(u):
            k_win, q_win = win[0], win[1]
            t, j = u // NG, u % NG
            hmask = []
            for i in range(G):
                l0 = ((j * G + i) * Dh) % L
                if l0 + Dh <= L:
                    hmask.append((lane >= l0) & (lane < l0 + Dh))
                else:
                    hmask.append((lane >= l0) | (lane < l0 + Dh - L))
            cs = slice(j * L, (j + 1) * L)
            ms = []
            for b in range(G):
                r0 = t * QT + b * QB
                qg = _u32(q_win[r0:r0 + QB, cs])
                qm = _b16(jnp.concatenate(
                    [jnp.where(hmask[(c - b) % G], qg, jnp.uint32(0)) for c in range(G)],
                    axis=0))
                c1 = cmin(t, b)
                kparts = [k_win[r0 + W:r0 + W + QB, cs]]
                if c1 < nc:
                    kparts.append(k_win[r0 + c1 * QB:r0 + W, cs])
                if not first:
                    kparts.insert(0, k_win[r0:r0 + QB, cs])
                sc = lax.dot_general(jnp.concatenate(kparts, axis=0), qm, _NT,
                                     preferred_element_type=f32)
                if first:
                    parts = [jnp.where(tri, NEG, sc[0:QB])]
                    if c1 < nc:
                        parts.append(sc[QB:])
                else:
                    parts = [jnp.where(tri, sc[0:QB], sc[QB:2 * QB]), sc[2 * QB:]]
                sc = jnp.concatenate(parts, axis=0)
                s_scrs[(u % NB) * G + b][zw, 0:sc.shape[0]] = sc
                ms.append(jnp.max(sc, axis=0, keepdims=True))
                fence[u, b] = jnp.broadcast_to(ms[b], (8, QT))
            for b in range(G):
                i = (u % NB) * G + b
                rows = (nc - cmin(t, b) + 1) * QB
                p_w[u % NB][0:rows, b * L:(b + 1) * L] = jnp.exp2(
                    s_scrs[i][zr, 0:rows] - ms[b]).astype(bf16)

        def pv(u):
            vt_win = win[2]
            t, j = u // NG, u % NG
            cols = slice(t * QT, (t + 1) * QT)
            p_scr = [p_r[u % NB].at[:, b * L:(b + 1) * L] for b in range(G)]
            fu = u + LAG - 1
            if fu < nu:
                p_w[u % NB][W:W + 16, 0:L] = _b16(_u32(fence[fu, G - 1]))

            def chunk(b, c):
                if c == nc:
                    pm = _u32(p_scr[b][0:QB])
                    return pm if first else pm & tri_c
                if c == 0 and not first:
                    return _u32(p_scr[b][0:QB]) & tri_a
                c1 = cmin(t, b)
                if c < c1:
                    return None
                return _u32(p_scr[b][(c - c1 + 1) * QB:(c - c1 + 2) * QB])

            def sel(msk, a, b):
                if a is None and b is None:
                    return None
                z = jnp.uint32(0)
                return jnp.where(msk, z if a is None else a, z if b is None else b)

            rows_per_head = [[] for _ in range(G)]
            for r in range(3 * QT // QB):
                xs = [chunk(b, r - b) if 0 <= r - b <= nc else None for b in range(G)]
                ys = [sel(bit0, xs[(m + 1) % G], xs[m]) for m in range(G)]
                zs = [sel(bit1, ys[(m + 2) % G], ys[m]) for m in range(G)]
                for i in range(G):
                    rows_per_head[i].append(zs[(-i) % G])

            os_ = [None] * G
            for c in range(2 - t if first else 0, 3):
                for i in range(G):
                    hd = j * G + i
                    pc = _b16(jnp.concatenate(rows_per_head[i][c * G:(c + 1) * G], axis=0))
                    oc = jnp.dot(vt_win[t + c, hd * VR:(hd + 1) * VR, :], pc,
                                 precision=lax.Precision.DEFAULT,
                                 preferred_element_type=f32)
                    os_[i] = oc if os_[i] is None else os_[i] + oc
            pend = None
            for i in range(G):
                c0 = (j * G + i) * Dh
                o = os_[i]
                r1 = 23 if c0 % 8 == 0 else 0
                o = o * (1.0 / o[r1:r1 + 1, :])
                if i:
                    o = pltpu.roll(o, QT - QB * i, 1)
                if c0 % 8 == 0:
                    ot_scr[c0:c0 + 16, cols] = o[0:16]
                    pend = o[16:24]
                else:
                    ot_scr[c0 - 4:c0 + 4, cols] = jnp.where(row8 < 4, pend, o[0:8])
                    ot_scr[c0 + 4:c0 + 20, cols] = o[8:24]
            if j == NG - 1:
                on_scr[cols, :] = ot_scr[:, cols].T.astype(bf16)

        def attention(items, pos, tail):
            assert len(items) == len(pos)
            done = 0
            tail = list(tail)
            for m in range(nu + LAG):
                if m < nu:
                    scores(m)
                if m >= LAG:
                    pv(m - LAG)
                if m < nu:
                    while done < len(items) and pos[done] <= m:
                        items[done]()
                        done += 1
                elif tail and m < nu + LAG - 1:
                    tail.pop(0)()
            for it in tail:
                it()

        def seq(*fns):
            def run():
                for fn in fns:
                    fn()
            return run

        V0 = lambda r0, r1, c0, c1: P(proj_v, xn0_scr, win, 0, r0, r1, c0, c1)
        V1 = lambda r0, r1, c0, c1: P(proj_v, xn_scr, win, T, r0, r1, c0, c1)
        QK = lambda *a: P(proj_qk, xn_scr, win, T, *a)
        if first:
            xcopy(0).start()
            for i in (0, 1, 2):
                wcopy(i).start()
            xcopy(1).start()
            for i in (3, 4):
                wcopy(i).start()
            xcopy(2).start()
            for i in (5, 6):
                wcopy(i).start()
            for i in range(3, n):
                xcopy(i).start()
            w0 = windows(zw)
            xcopy(0).wait()
            ln1(xn0_scr, xt(0))
            wcopy(0).wait()
            proj_qk(xn0_scr, w0, 0, 0, T, 0, 4)
            wcopy(1).wait()
            proj_qk(xn0_scr, w0, 0, 0, T, 4, 8)
            wcopy(2).wait()
            proj_v(xn0_scr, w0, 0, 0, T, 0, 2)
            proj_qk(xn0_scr, w0, 0, 0, T, 8, 10)
            xcopy(1).wait()
            wcopy(3).wait()
            blocks.clear()
            ln1(xn_scr, xt(1))
            attention([V0(0, h, 2, 4), V0(h, T, 2, 4), seq(V0(0, h, 4, 5), V0(h, T, 4, 5)),
                       QK(0, h, 0, 2), V1(0, h, 0, 2), V1(0, h, 2, 4), V1(h, T, 0, 2),
                       V1(h, T, 2, 4),
                       seq(V1(0, h, 4, 5), V1(h, T, 4, 5), QK(h, T, 0, 2)),
                       QK(0, h, 2, 6)], FPOS,
                      [QK(h, T, 2, 6), QK(0, h, 6, 10), QK(h, T, 6, 10)])
            for i in (4, 5, 6):
                wcopy(i).wait()
            xcopy(2).wait()
        elif not last:
            deps = ln1(xn_scr, xt(tile0 + 1))
            oproj(0, xt(tile0 - 1), 0, h, deps[:1], (3,))
            oproj(0, xt(tile0 - 1), h, T, deps[1:], (0, 2))
            attention(ffn_items(0, tile0 - 1), SPOS,
                      [V1(0, T, 0, 4), seq(V1(0, T, 4, 5), QK(0, T, 0, 3)),
                       QK(0, T, 3, 10, 4)])
            ocopy(tile0 - 1).start()

            @pl.when(tile0 + 2 < n)
            def _():
                xcopy(tile0 + 2).wait()
        else:
            oproj(0, xt(n - 2), 0, h)
            oproj(0, xt(n - 2), h, T)
            items = ffn_items(0, n - 2)
            items.insert(11, P(oproj, 1, xt(n - 1), 0, h))
            fin = ffn_items(1, n - 1)
            attention(items, LPOS, fin[:4])
            oproj(1, xt(n - 1), h, T)
            for it in fin[4:11]:
                it()
            ocopy(n - 2).start()
            for it in fin[11:]:
                it()
            ocopy(n - 1).start()
            for i in range(n):
                ocopy(i).wait()

    lax.cond((step > 0) & (step < n - 1), P(body, False, False),
             lambda: lax.cond(step == 0, P(body, True, False), P(body, False, True)))


@jax.jit
def pallas_sequential_preLN__sliding_block__dense_activation_relu__prompt_kernel(
    A_x: jax.Array,
    A_wqkv: jax.Array,
    A_wo: jax.Array,
    B_x: jax.Array,
    B_w1: jax.Array,
    B_w2: jax.Array,
):
    B, S, D = A_x.shape
    Dff = B_w1.shape[1]
    Dh = D // H
    assert B == 1 and S % T == 0 and S // T >= 3 and T == W
    assert (D, Dh, Dff) == (640, 20, 1536)
    n = S // T
    u32, f32 = jnp.uint32, jnp.float32

    hbm = pl.BlockSpec(memory_space=pl.ANY)
    return pl.pallas_call(
        functools.partial(_kernel, D=D, Dh=Dh, Dff=Dff, n=n),
        grid=(n,),
        in_specs=[hbm] * 5,
        out_specs=hbm,
        out_shape=jax.ShapeDtypeStruct((B, S, D), A_x.dtype),
        scratch_shapes=[
            pltpu.VMEM((S // 2, D), u32),
            pltpu.VMEM((S // 2, D), u32),
            pltpu.VMEM((D // 2, 3 * D), u32),
            pltpu.VMEM((D // 2, D), u32),
            pltpu.VMEM((D // 2, Dff), u32),
            pltpu.VMEM((Dff // 2, D), u32),
            pltpu.VMEM(((S + W + T) // 2, NG * L), u32),
            pltpu.VMEM(((S + W + T) // QT, H * VR, QT), f32),
            pltpu.VMEM((D, T), f32),
            pltpu.VMEM(((S + T) // 2, NG * L), u32),
            pltpu.VMEM((2, T, D), f32),
            pltpu.VMEM((2, T // 2, D), u32),
            pltpu.VMEM((3, T // 2, D), u32),
            pltpu.VMEM((T // 2, Dff), u32),
            pltpu.SemaphoreType.DMA((7,)),
            pltpu.SemaphoreType.DMA((n,)),
            pltpu.SemaphoreType.DMA((n,)),
        ] + [pltpu.VMEM((1, W, QT), f32)] * (NB * G)
          + [pltpu.VMEM((1, W // 2 + 8, G * QT), u32)] * NB,
        compiler_params=pltpu.CompilerParams(
            dimension_semantics=("arbitrary",),
            vmem_limit_bytes=100 * 1024 * 1024,
        ),
        name="preln_swa_ffn",
    )(A_x, A_wqkv, A_wo, B_w1, B_w2)
```
